```python
import jax
import jax.numpy as jnp

def _softmax(x, axis=-1):
    return jax.nn.softmax(x, axis=axis)
def _gelu(x):
    return jax.nn.gelu(x, approximate=True)
def _silu(x):
    return jax.nn.silu(x)
def _sigmoid(x):
    return jax.nn.sigmoid(x)
def _layernorm(x, axis=-1, eps=1e-5):
    m = jnp.mean(x, axis=axis, keepdims=True)
    v = jnp.var(x, axis=axis, keepdims=True)
    return (x - m) / jnp.sqrt(v + eps)
def _scatter_add(tgt, idx, src, axis=0):
    return tgt.at[idx].add(src)
def _segment_sum(src, seg, n):
    return jax.ops.segment_sum(src, seg, n)
class _Rng:
    def __init__(self, key):
        self._k = key
    def _next(self):
        self._k, sub = jax.random.split(self._k)
        return sub
    def normal(self, shape):
        return jax.random.normal(self._next(), shape, dtype=jnp.bfloat16)
    def randint(self, lo, hi, shape):
        return jax.random.randint(self._next(), shape, lo, hi, dtype=jnp.int32)
    def uniform(self, shape, lo=0.0, hi=1.0):
        return jax.random.uniform(self._next(), shape, jnp.bfloat16, lo, hi)
    def permutation(self, n):
        return jax.random.permutation(self._next(), n)


kernel_name = 'recurrent_scan__compressed_kv_cla__dense_activation_gelu__decode'

def setup_inputs():
    _rng = _Rng(jax.random.key(int.from_bytes(__import__("os").urandom(4), "little")))
    _w = (lambda a: (lambda t: t.astype(jnp.bfloat16) if jnp.issubdtype(t.dtype, jnp.floating) else t)(jnp.asarray(a)))
    def _A_setup():
        B, H, Sq, Sk, D, M = 2, 32, 1, 16384, 128, 512
        Dc = 4 * D
        return {
            "x": _w((lambda *s: _rng.normal(s) * 0.05)(B, Sq, M)),
            "c_kv": _w((lambda *s: _rng.normal(s) * 0.05)(B, Sk, Dc)),
            "w_q": _w((lambda *s: _rng.normal(s) * 0.05)(M, H, D) * (M ** -0.5)),
            "w_uk": _w((lambda *s: _rng.normal(s) * 0.05)(Dc, H, D) * (Dc ** -0.5)),
            "w_uv": _w((lambda *s: _rng.normal(s) * 0.05)(Dc, H, D) * (Dc ** -0.5)),
            "w_o": _w((lambda *s: _rng.normal(s) * 0.05)(H, D, M) * ((H * D) ** -0.5)),
        }
    _A_in = _A_setup()

    def _B_setup():
        B, S, D, F = 2, 1, 512, 1792
        return {
            "x": _w((lambda *s: _rng.normal(s) * 0.05)(B, S, D)),
            "w1": _w((lambda *s: _rng.normal(s) * 0.05)(D, F) * (D ** -0.5)),
            "b1": _w((lambda *s: _rng.normal(s) * 0.05)(F) * 0.01),
            "w2": _w((lambda *s: _rng.normal(s) * 0.05)(F, D) * (F ** -0.5)),
            "b2": _w((lambda *s: _rng.normal(s) * 0.05)(D) * 0.01),
        }
    _B_in = _B_setup()

    return {
        "A_x": _A_in["x"],
        "A_c_kv": _A_in["c_kv"],
        "A_w_q": _A_in["w_q"],
        "A_w_uk": _A_in["w_uk"],
        "A_w_uv": _A_in["w_uv"],
        "A_w_o": _A_in["w_o"],
        "B_x": _B_in["x"],
        "B_w1": _B_in["w1"],
        "B_b1": _B_in["b1"],
        "B_w2": _B_in["w2"],
        "B_b2": _B_in["b2"],
    }

def reference(A_x, A_c_kv, A_w_q, A_w_uk, A_w_uv, A_w_o, B_x, B_w1, B_b1, B_w2, B_b2):
    def _A_ref(x, c_kv, w_q, w_uk, w_uv, w_o):
        B, Sq, M = x.shape[0], x.shape[1], x.shape[2]
        Sk = c_kv.shape[1]
        H, D = w_q.shape[1], w_q.shape[2]
        q = jnp.einsum("bqm,mhd->bhqd", x, w_q)
        k = jnp.einsum("bkc,chd->bhkd", c_kv, w_uk)
        v = jnp.einsum("bkc,chd->bhkd", c_kv, w_uv)
        scores = jnp.einsum("bhqd,bhkd->bhqk", q, k) * (D ** -0.5)
        off = Sk - Sq
        qi = jnp.arange(Sq)[:, None]
        kj = jnp.arange(Sk)[None, :]
        cmask = kj <= (qi + off)
        scores = jnp.where(cmask[None, None], scores, -1e9)
        p = _softmax(scores, axis=-1)
        ctx = jnp.einsum("bhqk,bhkd->bhqd", p, v)
        return jnp.einsum("bhqd,hdm->bqm", ctx, w_o)

    def _B_ref(x, w1, b1, w2, b2):
        h = jnp.einsum("bsd,df->bsf", x, w1) + b1
        h = _gelu(h)
        return jnp.einsum("bsf,fd->bsd", h, w2) + b2

    x = A_x
    xn = _layernorm(x, axis=-1)
    s = _A_ref(xn, A_c_kv, A_w_q, A_w_uk, A_w_uv, A_w_o)
    g = _silu(_B_ref(xn, B_w1, B_b1, B_w2, B_b2))
    return x + s * g
```

```python
import jax
import jax.numpy as jnp
from jax import lax
import jax.experimental.pallas as pl
import jax.experimental.pallas.tpu as pltpu

F32 = jnp.float32
BF16 = jnp.bfloat16
U32 = jnp.uint32
B, H, SK, D, M, DC, F = 2, 32, 16384, 128, 512, 512, 1792
LOG2E = 1.4426950408889634
NT = (((1,), (1,)), ((), ()))
T_W1, T_Q, T_UK, T_C, T_W2, T_UV, T_O, T_END = 0, 16, 48, 80, 336, 350, 382, 414
SEGS = (T_W1, T_Q, T_UK, T_C, T_W2, T_UV, T_O, T_END)


def make_kernel(LAG=6, LAND=18, cmode='b8', nosem=True, nobc=True, dma_only=False, prof=False, A0=5):

    def _kernel(x_hbm, ckv_hbm, wq_hbm, wuk_hbm, wuv_hbm, wo_hbm, w1_hbm, b1_hbm, w2_hbm, b2_hbm,
                o_ref,
                x_buf, b1_buf, b2_buf, c_buf, wq_buf, wuk_buf, wuv_buf, wo_buf, w1_buf,
                coef_ref, q_ref, qa_ref, acc_ref, m_ref, l_ref, ctx_ref, lhs_ref,
                sem_g, sem_o, sem_small):

        def al(v, k):
            return v if isinstance(v, int) else pl.multiple_of(v, k)

        def gsem(seg, g):
            return sem_g.at[({T_Q: 0, T_UK: 4, T_C: 0, T_UV: 0}[seg] + g) & 7]

        def copy(seg, i, u):
            if seg in (T_Q, T_UK, T_UV):
                hbm, buf = {T_Q: (wq_hbm, wq_buf), T_UK: (wuk_hbm, wuk_buf), T_UV: (wuv_hbm, wuv_buf)}[seg]
                return pltpu.make_async_copy(hbm.at[:, u, pl.ds(i * 2, 2)], buf.at[:, u, pl.ds(i * 2, 2)],
                                             gsem(seg, i >> 3))
            if seg == T_C:
                if cmode == 'b8':
                    q, row = (i >> 7) * 4 + (i & 1) * 2 + u // 2, (u % 2) * 1024 + ((i & 127) >> 1) * 16
                elif cmode == 'b4':
                    q, row = (i >> 7) * 4 + u, (i & 127) * 16
                elif cmode == 'c8':
                    q, row = (i >> 7) * 4 + u, (i & 1) * 1024 + ((i & 127) >> 1) * 16
                elif cmode == 'c16':
                    q, row = (i >> 7) * 4 + u, (i & 3) * 512 + ((i & 127) >> 2) * 16
                return pltpu.make_async_copy(ckv_hbm.at[q, :, pl.ds(al(row, 16), 16)], c_buf.at[i, u],
                                             gsem(seg, i >> 3))
            if seg == T_W1:
                o = al((((i & 1) * 4 + u) * 8 + (i >> 1)) * 8, 8)
                return pltpu.make_async_copy(w1_hbm.at[pl.ds(o, 8)], w1_buf.at[pl.ds(o, 8)], sem_small.at[2])
            if seg == T_W2:
                return pltpu.make_async_copy(w2_hbm.at[:, u, pl.ds(al(i * 16, 16), 16)], c_buf.at[256 + i, u],
                                             sem_small.at[2])
            return pltpu.make_async_copy(wo_hbm.at[:, u, pl.ds(al(i * 16, 16), 16)], wo_buf.at[i, u], sem_o.at[i])

        def seg_of(t):
            return max(s for s in SEGS if s <= t)

        def wait(ref, sem):
            if prof:
                with jax.named_scope('W'):
                    pltpu.make_async_copy(ref, ref, sem).wait()
            else:
                pltpu.make_async_copy(ref, ref, sem).wait()

        pos = [0]

        def point(n0, j=0):
            def go():
                s1 = seg_of(n0)
                if s1 != T_END:
                    for u in range(3):
                        copy(s1, n0 - s1 + j, u).start(priority=1)
                if 0 <= n0 - LAG < T_END:
                    s0 = seg_of(n0 - LAG)
                    copy(s0, n0 - LAG - s0 + j, 3).start(priority=0)
            if prof == 2:
                with jax.named_scope('w'):
                    go()
            else:
                go()

        def loop(trips, body, carry=None, per=1):
            lo, hi = pos[0], pos[0] + trips * per
            edges = {c for s in SEGS for c in (s, s + LAG) if lo < c < hi}
            cuts = {0, trips} | {(c - lo) // per for c in edges} | {-((lo - c) // per) for c in edges}
            cuts = sorted(cuts)
            for a, b in zip(cuts[:-1], cuts[1:]):
                def it(k, carry, a=a):
                    return body(a + k, lambda v: point(lo + a * per + v, k * per), carry)

                carry = it(0, carry) if b - a == 1 and per > 1 else lax.fori_loop(0, b - a, it, carry)
            pos[0] = hi
            return carry

        def tick1():
            point(pos[0])
            pos[0] += 1

        def landed(t):
            n = t + LAG + LAND - pos[0]
            if n > 0:
                loop(n, lambda k, tick, c: tick(0))

        x_copy = pltpu.make_async_copy(x_hbm, x_buf, sem_small.at[0])
        b1_copy = pltpu.make_async_copy(b1_hbm, b1_buf, sem_small.at[1])
        b2_copy = pltpu.make_async_copy(b2_hbm, b2_buf, sem_small.at[1])
        for i in range(LAG + 1):
            tick1()
            if i == 1:
                x_copy.start()
                b1_copy.start()
                b2_copy.start()
        landed(0)

        x_copy.wait()
        x = x_buf[...].astype(F32)
        xc = x - jnp.mean(x, axis=-1, keepdims=True)
        var = jnp.mean(xc * xc, axis=-1, keepdims=True)
        xn = (xc * lax.rsqrt(var + 1e-5)).astype(BF16)

        def pack(lo, hi):
            lo = lax.bitcast_convert_type(lo.astype(BF16).astype(F32), U32)
            hi = lax.bitcast_convert_type(hi.astype(BF16).astype(F32), U32)
            return (lo >> 16) | hi

        xw = jnp.broadcast_to(pack(xn[0:1], xn[1:2]), (H, M))
        for j in range(4):
            coef_ref[j] = xw[:, j * 128:(j + 1) * 128]

        landed(T_Q)
        b1_copy.wait()
        b2_copy.wait()
        wait(w1_buf, sem_small.at[2])
        hs = []
        for o in range(0, F, 256):
            tick1()
            hs.append(jnp.dot(xn, w1_buf[:, o:o + 256], preferred_element_type=F32))
        h = jnp.concatenate(hs, axis=1) + b1_buf[...].astype(F32).reshape(1, F)
        h = jax.nn.gelu(h, approximate=True).astype(BF16)

        lane = lax.broadcasted_iota(jnp.int32, (16, 128), 1)
        diag = (lane % 16) == lax.broadcasted_iota(jnp.int32, (16, 128), 0)

        def head_contract(seg, buf):
            def lhs(k):
                g, r = k >> 3, k & 7
                a = []
                for hg in range(2):
                    cw = coef_ref[r >> 1, hg * 16:(hg + 1) * 16, :]
                    for t in range(2):
                        rep = jnp.take_along_axis(cw, lane // 16 + ((r & 1) * 64 + g * 16 + t * 8), axis=1)
                        a.append(jnp.where(diag, rep, jnp.uint32(0)))
                return tuple(a)

            def body(k, tick, carry):
                out, a = carry
                g, r = k >> 3, k & 7
                pl.when(r == 0)(lambda: wait(buf.at[:, :, pl.ds(g * 16, 16)], gsem(seg, g)))
                tick(0)
                if dma_only:
                    return carry
                res = []
                for hg in range(2):
                    w = buf[r >> 2, r & 3, pl.ds(g * 16, 16), hg * 16:(hg + 1) * 16, :].reshape(256, D)
                    sel = pltpu.bitcast(jnp.concatenate(a[2 * hg:2 * hg + 2], axis=1), BF16)
                    res.append(out[hg] + jnp.dot(sel, w, preferred_element_type=F32))
                return tuple(res), lhs((k + 1) & 31)

            first = lhs(0)
            landed(seg + 8)
            return loop(32, body, ((jnp.zeros((32, D), F32), jnp.zeros((32, D), F32)), first))[0]

        q = head_contract(T_Q, wq_buf)
        q = [v.astype(BF16) for v in q]

        lane32 = lax.broadcasted_iota(jnp.int32, (32, 128), 1)
        pick = (lane32 % 8) * 16 + lax.broadcasted_iota(jnp.int32, (32, 128), 0) // 2
        q_ref[...] = jnp.zeros(q_ref.shape, F32)

        def qa_extract(k, res):
            g, r = k >> 3, k & 7
            for hg in range(2):
                val = q_ref[r >> 1, hg * 32:(hg + 1) * 32, :]
                for t in range(2):
                    rep = jnp.take_along_axis(res[hg][:, t * 128:(t + 1) * 128], pick, axis=1)
                    val = jnp.where(lane32 // 8 == (r & 1) * 8 + g * 2 + t, rep, val)
                q_ref[r >> 1, hg * 32:(hg + 1) * 32, :] = val

        def qa_body(k, tick, prev):
            g, r = k >> 3, k & 7
            pl.when(r == 0)(lambda: wait(wuk_buf.at[:, :, pl.ds(g * 16, 16)], gsem(T_UK, g)))
            tick(0)
            if dma_only:
                return prev
            res = []
            for hg in range(2):
                w = wuk_buf[r >> 2, r & 3, pl.ds(g * 16, 16), hg * 16:(hg + 1) * 16, :].reshape(256, D)
                res.append(lax.dot_general(q[hg], w, NT, preferred_element_type=F32))
            qa_extract((k + 31) & 31, prev)
            return tuple(res)

        landed(T_UK + 8)
        qa_extract(31, loop(32, qa_body, (jnp.zeros((32, 256), F32), jnp.zeros((32, 256), F32))))
        for j in range(4):
            for b in range(B):
                qa_ref[b * H:(b + 1) * H, j * 128:(j + 1) * 128] = (
                    q_ref[j, pl.ds(b, H, stride=2), :] * (D ** -0.5 * LOG2E)).astype(BF16)

        m_ref[...] = jnp.full((B * H, 128), -jnp.inf, F32)
        l_ref[...] = jnp.zeros((B * H, 128), F32)
        acc_ref[...] = jnp.zeros((B * H, DC), F32)

        def attend(g, tick, _):
            wait(c_buf.at[pl.ds(g * 8, 8)], gsem(T_C, g))
            hrows = pl.ds(al((g >> 4) * H, H), H)

            def tiles(t):
                return c_buf[pl.ds(g * 8 + 2 * t, 2)].reshape(256, DC)

            if dma_only:
                for v in range(8):
                    tick(v)
                return
            qa = qa_ref[hrows, :]
            sc = []
            for t in range(4):
                tick(t)
                sc.append(lax.dot_general(qa, tiles(t), NT, preferred_element_type=F32))
            sc = jnp.concatenate(sc, axis=1)
            m_prev = m_ref[hrows, :]
            m_new = jnp.maximum(m_prev, jnp.max(sc, axis=1, keepdims=True))
            p = jnp.exp2(sc - m_new[:, :1])
            alpha = jnp.exp2(m_prev - m_new)
            l_ref[hrows, :] = alpha * l_ref[hrows, :] + jnp.sum(p, axis=1, keepdims=True)
            m_ref[hrows, :] = m_new
            p = p.astype(BF16)
            acc = acc_ref[hrows, :] * alpha[:, :1]
            for t in range(4):
                tick(4 + t)
                acc = acc + jnp.dot(p[:, t * 256:(t + 1) * 256], tiles(t), preferred_element_type=F32)
            acc_ref[hrows, :] = acc

        landed(T_C + 8)
        loop(32, attend, per=8)
        pc = acc_ref[...] / l_ref[...][:, :1]
        pw = pack(pc[:H], pc[H:])
        for j in range(4):
            coef_ref[j] = pw[:, j * 128:(j + 1) * 128]

        landed(T_UV)
        wait(c_buf.at[pl.ds(256, 14)], sem_small.at[2])
        gg = b2_buf[...].astype(F32).reshape(1, M)
        for p in range(2):
            tick1()
            w = jnp.concatenate([c_buf[pl.ds(256, 14), u, p].reshape(224, M) for u in range(4)], axis=0)
            gg = gg + jnp.dot(h[:, p * 896:(p + 1) * 896], w, preferred_element_type=F32)
        gate = gg * jax.nn.sigmoid(gg)

        ctx = head_contract(T_UV, wuv_buf)
        ctx_ref[0:32, :] = ctx[0]
        ctx_ref[32:64, :] = ctx[1]

        lane8 = lax.broadcasted_iota(jnp.int32, (8, 128), 1)
        reg = lax.broadcasted_iota(jnp.int32, (8, 128), 0)
        slot = (lane8 // 16) == (reg % 4) * 2 + reg // 4
        for hh in range(4):
            for b in range(B):
                rows = ctx_ref[pl.ds(2 * hh + b, 8, stride=8), :]
                for dd in range(8):
                    rep = jnp.take_along_axis(rows, lane8 % 16 + dd * 16, axis=1)
                    lhs_ref[hh * 8 + dd, pl.ds(b, 1), :] = jnp.sum(jnp.where(slot, rep, 0.0), axis=0, keepdims=True)

        def s_tiles(s, i, n):
            a = jnp.concatenate([lhs_ref[i + t] for t in range(n)], axis=1).astype(BF16)
            return s + jnp.dot(a, wo_buf[i:i + n].reshape(128 * n, M), preferred_element_type=F32)

        s = jnp.zeros((B, M), F32)
        i = done = 0
        while done < 32:
            want = max(i + 1, min(pos[0] - LAG - T_O - A0 + 1, 32)) if i < 32 else 32
            while i < want:
                while pos[0] - LAG <= T_O + i:
                    tick1()
                wait(wo_buf.at[i], sem_o.at[i])
                i += 1
            tick1()
            n = min(i - done, 3)
            s = s_tiles(s, done, n)
            done += n
        assert pos[0] - LAG >= T_END
        o_ref[...] = (x + s * gate).astype(BF16)

    def fn(A_x, A_c_kv, A_w_q, A_w_uk, A_w_uv, A_w_o, B_x, B_w1, B_b1, B_w2, B_b2):
        wshape = (2, 4, 64, H, D)
        out = pl.pallas_call(
            _kernel,
            out_shape=jax.ShapeDtypeStruct((B, M), BF16),
            in_specs=[pl.BlockSpec(memory_space=pltpu.HBM)] * 10,
            out_specs=pl.BlockSpec(memory_space=pltpu.VMEM),
            scratch_shapes=[
                pltpu.VMEM((B, M), BF16), pltpu.VMEM((F,), BF16), pltpu.VMEM((M,), BF16),
                pltpu.VMEM((256 + 14, 4, 2, 16, DC), BF16),
                pltpu.VMEM(wshape, BF16), pltpu.VMEM(wshape, BF16), pltpu.VMEM(wshape, BF16),
                pltpu.VMEM((32, 4, 2, 16, M), BF16), pltpu.VMEM((M, F), BF16),
                pltpu.VMEM((4, H, 128), U32), pltpu.VMEM((4, B * H + 8, 128), F32),
                pltpu.VMEM((B * H, DC), BF16), pltpu.VMEM((B * H, DC), F32),
                pltpu.VMEM((B * H, 128), F32), pltpu.VMEM((B * H, 128), F32),
                pltpu.VMEM((B * H + 8, D), F32), pltpu.VMEM((32, B, 128), F32),
                pltpu.SemaphoreType.DMA((8,)), pltpu.SemaphoreType.DMA((32,)), pltpu.SemaphoreType.DMA((3,)),
            ],
            compiler_params=pltpu.CompilerParams(vmem_limit_bytes=100 * 1024 * 1024, disable_semaphore_checks=nosem,
                                                 disable_bounds_checks=nobc),
        )(A_x.reshape(B, M), A_c_kv.reshape(8, 2, 2048, DC), A_w_q.reshape(wshape), A_w_uk.reshape(wshape),
          A_w_uv.reshape(wshape), A_w_o.reshape(2, 4, 512, M), B_w1, B_b1, B_w2.reshape(2, 4, 224, M), B_b2)
        return out.reshape(B, 1, M)

    return fn


@jax.jit
def pallas_recurrent_scan__compressed_kv_cla__dense_activation_gelu__decode_kernel(
    A_x, A_c_kv, A_w_q, A_w_uk, A_w_uv, A_w_o, B_x, B_w1, B_b1, B_w2, B_b2
):
    return make_kernel(LAG=8, LAND=16)(A_x, A_c_kv, A_w_q, A_w_uk, A_w_uv, A_w_o, B_x, B_w1, B_b1, B_w2, B_b2)
```

```python
import jax
import jax.numpy as jnp
from jax import lax
import jax.experimental.pallas as pl
import jax.experimental.pallas.tpu as pltpu

F32 = jnp.float32
BF16 = jnp.bfloat16
U32 = jnp.uint32
B, H, SK, D, M, DC, F = 2, 32, 16384, 128, 512, 512, 1792
LOG2E = 1.4426950408889634
NT = (((1,), (1,)), ((), ()))
T_W1, T_Q, T_UK, T_C, T_W2, T_UV, T_O, T_END = 0, 16, 48, 80, 336, 350, 382, 414


def make_kernel(pat=(1, 0, 1, 0), LAG=13, LEAD=28, pair=0, NV=2, A0=5, nosem=True, nobc=True, dma_only=False, prof=False,
                tail_groups=(8, 8, 4, 2, 2, 1, 1, 1, 1, 1, 1), xat=1, dummy=0, DV=0):
    SEGS = (T_W1, T_Q) + (() if pair else (T_UK,)) + (T_C, T_W2, T_UV, T_O, T_END)
    tail_groups = list(tail_groups)
    while sum(tail_groups) > 32 - NV:
        tail_groups.pop()
    tail_groups += [1] * (32 - NV - sum(tail_groups))
    o_off = [sum(tail_groups[:i]) for i in range(len(tail_groups) + 1)]

    def _kernel(x_hbm, ckv_hbm, wq_hbm, wuk_hbm, wuv_hbm, wo_hbm, w1_hbm, b1_hbm, w2_hbm, b2_hbm,
                o_ref,
                x_buf, b1_buf, b2_buf, c_buf, wq_buf, wuk_buf, wuv_buf, wo_buf, w1_buf, w2_buf,
                coef_ref, q_ref, qa_ref, acc_ref, m_ref, l_ref, ctx_ref, lhs_ref, col_ref, pad_buf,
                sem_g, sem_o, sem_v, sem_small):

        def al(v, k):
            return v if isinstance(v, int) else pl.multiple_of(v, k)

        def gsem(seg, g):
            return sem_g.at[({T_Q: 0, T_UK: 4, T_C: 8, T_UV: 8}[seg] + g) & 15]

        def copy(seg, i0, j, u):
            i = i0 + j
            if pair and seg == T_Q:
                seg, i = (T_Q, T_UK)[i0 & 1], i >> 1
            if seg in (T_Q, T_UK, T_UV):
                hbm, buf = {T_Q: (wq_hbm, wq_buf), T_UK: (wuk_hbm, wuk_buf), T_UV: (wuv_hbm, wuv_buf)}[seg]
                return pltpu.make_async_copy(hbm.at[:, u, pl.ds(i * 2, 2)], buf.at[:, u, pl.ds(i * 2, 2)],
                                             gsem(seg, i >> 3))
            if seg == T_C:
                q, row = (i >> 7) * 4 + (i0 & 1) * 2 + u // 2, (u % 2) * 1024 + ((i & 127) >> 1) * 16
                return pltpu.make_async_copy(ckv_hbm.at[q, :, pl.ds(al(row, 16), 16)], c_buf.at[i, u],
                                             gsem(seg, i >> 3))
            if seg == T_W1:
                o = al((((i0 & 1) * 4 + u) * 8 + (i >> 1)) * 8, 8)
                return pltpu.make_async_copy(w1_hbm.at[pl.ds(o, 8)], w1_buf.at[pl.ds(o, 8)], sem_small.at[2])
            if seg == T_W2:
                o = pl.ds(al(i * 16, 16), 16)
                return pltpu.make_async_copy(w2_hbm.at[:, u, o], w2_buf.at[:, u, o], sem_small.at[2])
            if i >= 32 - NV:
                sem = sem_v.at[(i - 32 + NV) * 4 + u]
            else:
                sem = sem_o.at[max(k for k, o in enumerate(o_off) if o <= i)]
            return pltpu.make_async_copy(wo_hbm.at[:, u, pl.ds(i * 16, 16)], wo_buf.at[i, u], sem)

        def seg_of(t):
            return max(s for s in SEGS if s <= t)

        def wait(ref, sem):
            if prof:
                with jax.named_scope('W'):
                    pltpu.make_async_copy(ref, ref, sem).wait()
            else:
                pltpu.make_async_copy(ref, ref, sem).wait()

        pos = [0]
        pads = []

        def point(n0, j=0):
            for u in range(4):
                t = n0 if pat[u] else n0 - LAG
                if 0 <= t < T_END:
                    s = seg_of(t)
                    copy(s, t - s, j, u).start(priority=pat[u])
                elif dummy and pat[u] and n0 - LAG < T_END:
                    pads.append(pltpu.make_async_copy(b2_hbm, pad_buf.at[pl.ds(len(pads) * M, M)], sem_small.at[1]))
                    pads[-1].start(priority=1)

        def loop(trips, body, carry=None, per=8):
            lo, hi = pos[0], pos[0] + trips * per
            edges = {c for s in SEGS for c in (s, s + LAG) if lo < c < hi}
            cuts = {0, trips} | {(c - lo) // per for c in edges} | {-((lo - c) // per) for c in edges}
            cuts |= {k for k in range(trips) if lo + (k + 1) * per > T_O}
            cuts = sorted(cuts)
            for a, b in zip(cuts[:-1], cuts[1:]):
                def it(k, carry, a=a):
                    for v in range(per):
                        point(lo + a * per + v, k * per)
                    return body(a + k, carry)

                carry = it(0, carry) if b - a == 1 else lax.fori_loop(0, b - a, it, carry)
            pos[0] = hi
            return carry

        def advance(n):
            if n - pos[0] >= 8:
                loop((n - pos[0]) // 2, lambda k, c: None, per=2)
            while pos[0] < n:
                point(pos[0])
                pos[0] += 1

        x_copy = pltpu.make_async_copy(x_hbm, x_buf, sem_small.at[0])
        b1_copy = pltpu.make_async_copy(b1_hbm, b1_buf, sem_small.at[1])
        b2_copy = pltpu.make_async_copy(b2_hbm, b2_buf, sem_small.at[1])
        for i in range(LAG + 2):
            advance(i + 1)
            if i == xat:
                x_copy.start()
                b1_copy.start()
                b2_copy.start()
        advance(LEAD)

        x_copy.wait()
        x = x_buf[...].astype(F32)
        xc = x - jnp.mean(x, axis=-1, keepdims=True)
        var = jnp.mean(xc * xc, axis=-1, keepdims=True)
        xn = (xc * lax.rsqrt(var + 1e-5)).astype(BF16)

        def pack(lo, hi):
            lo = lax.bitcast_convert_type(lo.astype(BF16).astype(F32), U32)
            hi = lax.bitcast_convert_type(hi.astype(BF16).astype(F32), U32)
            return (lo >> 16) | hi

        coef_ref[...] = jnp.broadcast_to(pack(xn[0:1], xn[1:2]), (H, M))

        advance(T_Q + LEAD)
        b1_copy.wait()
        b2_copy.wait()
        wait(w1_buf, sem_small.at[2])
        h = jnp.dot(xn, w1_buf[...], preferred_element_type=F32) + b1_buf[...].astype(F32).reshape(1, F)
        h = jax.nn.gelu(h, approximate=True).astype(BF16)

        lane = lax.broadcasted_iota(jnp.int32, (16, 128), 1)
        diag = (lane % 16) == lax.broadcasted_iota(jnp.int32, (16, 128), 0)

        def head_contract(seg, buf, per):
            def body(g, out):
                wait(buf.at[:, :, pl.ds(g * 16, 16)], gsem(seg, g))
                if dma_only:
                    return out
                res = []
                for hg in range(2):
                    a = []
                    for r in range(8):
                        cw = coef_ref[hg * 16:(hg + 1) * 16, (r // 2) * 128:(r // 2 + 1) * 128]
                        for t in range(2):
                            rep = jnp.take_along_axis(cw, lane // 16 + ((r % 2) * 64 + g * 16 + t * 8), axis=1)
                            a.append(jnp.where(diag, rep, jnp.uint32(0)))
                    sel = pltpu.bitcast(jnp.concatenate(a, axis=1), BF16)
                    w = buf[:, :, pl.ds(g * 16, 16), hg * 16:(hg + 1) * 16, :].reshape(2048, D)
                    res.append(out[hg] + jnp.dot(sel, w, preferred_element_type=F32))
                return tuple(res)

            advance(seg + LEAD)
            return loop(4, body, (jnp.zeros((32, D), F32), jnp.zeros((32, D), F32)), per=per)

        q = [v.astype(BF16) for v in head_contract(T_Q, wq_buf, 16 if pair else 8)]

        lane32 = lax.broadcasted_iota(jnp.int32, (32, 128), 1)
        pick = (lane32 % 8) * 16 + lax.broadcasted_iota(jnp.int32, (32, 128), 0) // 2
        q_ref[...] = jnp.zeros(q_ref.shape, F32)

        def qa_body(g, _):
            wait(wuk_buf.at[:, :, pl.ds(g * 16, 16)], gsem(T_UK, g))
            if dma_only:
                return
            for hg in range(2):
                w = wuk_buf[:, :, pl.ds(g * 16, 16), hg * 16:(hg + 1) * 16, :].reshape(2048, D)
                res = lax.dot_general(q[hg], w, NT, preferred_element_type=F32)
                for j in range(4):
                    val = q_ref[j, hg * 32:(hg + 1) * 32, :]
                    for t in range(4):
                        rep = jnp.take_along_axis(res[:, (j * 4 + t) * 128:(j * 4 + t + 1) * 128], pick, axis=1)
                        val = jnp.where(lane32 // 8 == (t // 2) * 8 + g * 2 + t % 2, rep, val)
                    q_ref[j, hg * 32:(hg + 1) * 32, :] = val

        loop(4, qa_body, per=4 if pair else 8)
        for j in range(4):
            for b in range(B):
                qa_ref[b * H:(b + 1) * H, j * 128:(j + 1) * 128] = (
                    q_ref[j, pl.ds(b, H, stride=2), :] * (D ** -0.5 * LOG2E)).astype(BF16)

        m_ref[...] = jnp.full((B * H, 128), -jnp.inf, F32)
        l_ref[...] = jnp.zeros((B * H, 128), F32)
        acc_ref[...] = jnp.zeros((B * H, DC), F32)

        def attend(g, _):
            wait(c_buf.at[pl.ds(g * 8, 8)], gsem(T_C, g))
            if dma_only:
                return
            hrows = pl.ds(al((g >> 4) * H, H), H)
            c = c_buf[pl.ds(g * 8, 8)].reshape(1024, DC)
            sc = lax.dot_general(qa_ref[hrows, :], c, NT, preferred_element_type=F32)
            m_prev = m_ref[hrows, :]
            m_new = jnp.maximum(m_prev, jnp.max(sc, axis=1, keepdims=True))
            p = jnp.exp2(sc - m_new[:, :1])
            alpha = jnp.exp2(m_prev - m_new)
            l_ref[hrows, :] = alpha * l_ref[hrows, :] + jnp.sum(p, axis=1, keepdims=True)
            m_ref[hrows, :] = m_new
            pv = jnp.dot(p.astype(BF16), c, preferred_element_type=F32)
            acc_ref[hrows, :] = acc_ref[hrows, :] * alpha[:, :1] + pv

        assert pos[0] >= T_C + LEAD
        loop(32, attend)
        pc = acc_ref[...] / l_ref[...][:, :1]
        coef_ref[...] = pack(pc[:H], pc[H:])

        advance(T_UV + LEAD)
        wait(w2_buf, sem_small.at[2])
        gg = b2_buf[...].astype(F32).reshape(1, M) + jnp.dot(h, w2_buf[...].reshape(F, M), preferred_element_type=F32)
        gate = gg * jax.nn.sigmoid(gg)

        ctx = head_contract(T_UV, wuv_buf, 8)
        ctx_ref[0:32, :] = ctx[0]
        ctx_ref[32:64, :] = ctx[1]

        advance(min(pos[0] + 3, T_END))
        lane8 = lax.broadcasted_iota(jnp.int32, (8, 128), 1)
        reg = lax.broadcasted_iota(jnp.int32, (8, 128), 0)
        slot = (lane8 // 16) == (reg % 4) * 2 + reg // 4
        for hh in range(4):
            for b in range(B):
                rows = ctx_ref[pl.ds(2 * hh + b, 8, stride=8), :]
                for dd in range(8):
                    rep = jnp.take_along_axis(rows, lane8 % 16 + dd * 16, axis=1)
                    lhs_ref[hh * 8 + dd, pl.ds(b, 1), :] = jnp.sum(jnp.where(slot, rep, 0.0), axis=0, keepdims=True)
        for i in range(NV):
            for b in range(B):
                row = lhs_ref[32 - NV + i, pl.ds(b, 1), :].astype(BF16).astype(F32)
                col_ref[i, b] = jnp.broadcast_to(row, (128, 128)).T
        advance(T_END + (LAG if dummy else 0))

        s = jnp.zeros((B, M), F32)
        for k, n in enumerate(tail_groups):
            i = o_off[k]
            advance(T_O + i + n + LAG)
            wait(wo_buf.at[i:i + n], sem_o.at[k])
            advance(min(T_O + i + n + A0 + LAG, T_END + LAG, pos[0] + n + 1))
            a = jnp.concatenate([lhs_ref[i + t] for t in range(n)], axis=1).astype(BF16)
            s = s + jnp.dot(a, wo_buf[i:i + n].reshape(128 * n, M), preferred_element_type=F32)
        nxt = [(pos[0] - LAG - T_O) * 4]

        def top_up(j):
            while nxt[0] < min(j, 128):
                i, u = divmod(nxt[0], 4)
                if not pat[u]:
                    copy(T_O, i, 0, u).start(priority=0)
                nxt[0] += 1

        assert pos[0] >= T_END
        if not DV:
            top_up(128)
        if NV:
            base = x + s * gate
            acc = [jnp.zeros((8, M), F32)] * B
            for i in range(NV):
                for u in range(4):
                    j = (32 - NV + i) * 4 + u
                    top_up(j + 1)
                    wait(wo_buf.at[32 - NV + i, u], sem_v.at[i * 4 + u])
                    top_up(min(j + DV, nxt[0] + 2))
                    w = wo_buf[32 - NV + i, u].reshape(32, M).astype(F32)
                    for b in range(B):
                        col = jnp.concatenate([col_ref[i, b, u * 32:(u + 1) * 32, :]] * 4, axis=1)
                        pr = w * col
                        acc[b] = acc[b] + ((pr[0:8] + pr[8:16]) + (pr[16:24] + pr[24:32]))
            s = jnp.concatenate([jnp.sum(a, axis=0, keepdims=True) for a in acc], axis=0)
            o_ref[...] = (base + s * gate).astype(BF16)
        else:
            o_ref[...] = (x + s * gate).astype(BF16)
        for c in pads:
            c.wait()

    def fn(A_x, A_c_kv, A_w_q, A_w_uk, A_w_uv, A_w_o, B_x, B_w1, B_b1, B_w2, B_b2):
        wshape = (2, 4, 64, H, D)
        out = pl.pallas_call(
            _kernel,
            out_shape=jax.ShapeDtypeStruct((B, M), BF16),
            in_specs=[pl.BlockSpec(memory_space=pltpu.HBM)] * 10,
            out_specs=pl.BlockSpec(memory_space=pltpu.VMEM),
            scratch_shapes=[
                pltpu.VMEM((B, M), BF16), pltpu.VMEM((F,), BF16), pltpu.VMEM((M,), BF16),
                pltpu.VMEM((256, 4, 2, 16, DC), BF16),
                pltpu.VMEM(wshape, BF16), pltpu.VMEM(wshape, BF16), pltpu.VMEM(wshape, BF16),
                pltpu.VMEM((32, 4, 2, 16, M), BF16), pltpu.VMEM((M, F), BF16), pltpu.VMEM((2, 4, 224, M), BF16),
                pltpu.VMEM((H, DC), U32), pltpu.VMEM((4, B * H + 8, 128), F32),
                pltpu.VMEM((B * H, DC), BF16), pltpu.VMEM((B * H, DC), F32),
                pltpu.VMEM((B * H, 128), F32), pltpu.VMEM((B * H, 128), F32),
                pltpu.VMEM((B * H + 8, D), F32), pltpu.VMEM((32, B, 128), F32),
                pltpu.VMEM((max(NV, 1), B, 128, 128), F32), pltpu.VMEM((64 * M,), BF16),
                pltpu.SemaphoreType.DMA((16,)), pltpu.SemaphoreType.DMA((len(tail_groups),)),
                pltpu.SemaphoreType.DMA((max(4 * NV, 1),)), pltpu.SemaphoreType.DMA((3,)),
            ],
            compiler_params=pltpu.CompilerParams(vmem_limit_bytes=100 * 1024 * 1024, disable_semaphore_checks=nosem,
                                                 disable_bounds_checks=nobc),
        )(A_x.reshape(B, M), A_c_kv.reshape(8, 2, 2048, DC), A_w_q.reshape(wshape), A_w_uk.reshape(wshape),
          A_w_uv.reshape(wshape), A_w_o.reshape(2, 4, 512, M), B_w1, B_b1, B_w2.reshape(2, 4, 224, M), B_b2)
        return out.reshape(B, 1, M)

    return fn


@jax.jit
def pallas_recurrent_scan__compressed_kv_cla__dense_activation_gelu__decode_kernel(
    A_x, A_c_kv, A_w_q, A_w_uk, A_w_uv, A_w_o, B_x, B_w1, B_b1, B_w2, B_b2
):
    return make_kernel(NV=8, A0=6, DV=24)(A_x, A_c_kv, A_w_q, A_w_uk, A_w_uv, A_w_o, B_x, B_w1, B_b1, B_w2, B_b2)
```

```python
import jax
import jax.numpy as jnp
from jax import lax
import jax.experimental.pallas as pl
import jax.experimental.pallas.tpu as pltpu

F32 = jnp.float32
BF16 = jnp.bfloat16
U32 = jnp.uint32
B, H, SK, D, M, DC, F = 2, 32, 16384, 128, 512, 512, 1792
LOG2E = 1.4426950408889634
NT = (((1,), (1,)), ((), ()))
T_W1, T_Q, T_UK, T_C, T_W2, T_UV, T_O, T_END = 0, 16, 48, 80, 336, 350, 382, 414


def make_kernel(seq=((0, 0), (3, 13), (2, 0), (1, 12)), LEAD=28, pair=0, NV=8, A0=6, tk='rr', tn=0, epi=1, dma_only=False, prof=False,
                tail_groups=(8, 8, 4, 2, 2, 1, 1, 1, 1, 1, 1), xat=1, DV=24):
    LAG = max(l for _, l in seq)
    pat = [int(dict(seq)[u] == 0) for u in range(4)]
    rest = range(32 - tn, 32)
    order = [(u, i) for i in range(32 - tn) for u in range(4)] + {'rr': [(u, i) for i in rest for u in range(4)],
        '3+1': [(u, i) for i in rest for u in range(3)] + [(3, i) for i in rest],
        '2+1+1': [(u, i) for i in rest for u in range(2)] + [(u, i) for u in (2, 3) for i in rest]}[tk]
    assert tn <= NV
    SEGS = (T_W1, T_Q) + (() if pair else (T_UK,)) + (T_C, T_W2, T_UV, T_O, T_END)
    tail_groups = list(tail_groups)
    while sum(tail_groups) > 32 - NV:
        tail_groups.pop()
    tail_groups += [1] * (32 - NV - sum(tail_groups))
    o_off = [sum(tail_groups[:i]) for i in range(len(tail_groups) + 1)]

    def _kernel(x_hbm, ckv_hbm, wq_hbm, wuk_hbm, wuv_hbm, wo_hbm, w1_hbm, b1_hbm, w2_hbm, b2_hbm,
                o_ref,
                x_buf, b1_buf, b2_buf, c_buf, wq_buf, wuk_buf, wuv_buf, wo_buf, w1_buf, w2_buf,
                coef_ref, q_ref, qa_ref, acc_ref, m_ref, l_ref, ctx_ref, lhs_ref, col_ref,
                sem_g, sem_o, sem_v, sem_small):

        def al(v, k):
            return v if isinstance(v, int) else pl.multiple_of(v, k)

        def gsem(seg, g):
            return sem_g.at[({T_Q: 0, T_UK: 4, T_C: 8, T_UV: 8}[seg] + g) & 15]

        def copy(seg, i0, j, u):
            i = i0 + j
            if pair and seg == T_Q:
                seg, i = (T_Q, T_UK)[i0 & 1], i >> 1
            if seg in (T_Q, T_UK, T_UV):
                hbm, buf = {T_Q: (wq_hbm, wq_buf), T_UK: (wuk_hbm, wuk_buf), T_UV: (wuv_hbm, wuv_buf)}[seg]
                return pltpu.make_async_copy(hbm.at[:, u, pl.ds(i * 2, 2)], buf.at[:, u, pl.ds(i * 2, 2)],
                                             gsem(seg, i >> 3))
            if seg == T_C:
                q, row = (i >> 7) * 4 + (i0 & 1) * 2 + u // 2, (u % 2) * 1024 + ((i & 127) >> 1) * 16
                return pltpu.make_async_copy(ckv_hbm.at[q, :, pl.ds(al(row, 16), 16)], c_buf.at[i, u],
                                             gsem(seg, i >> 3))
            if seg == T_W1:
                o = al((((i0 & 1) * 4 + u) * 8 + (i >> 1)) * 8, 8)
                return pltpu.make_async_copy(w1_hbm.at[pl.ds(o, 8)], w1_buf.at[pl.ds(o, 8)], sem_small.at[2])
            if seg == T_W2:
                o = pl.ds(al(i * 16, 16), 16)
                return pltpu.make_async_copy(w2_hbm.at[:, u, o], w2_buf.at[:, u, o], sem_small.at[2])
            if i >= 32 - NV:
                sem = sem_v.at[(i - 32 + NV) * 4 + u]
            else:
                sem = sem_o.at[max(k for k, o in enumerate(o_off) if o <= i)]
            su, si = order[i * 4 + u]
            return pltpu.make_async_copy(wo_hbm.at[:, su, pl.ds(si * 16, 16)], wo_buf.at[i, u], sem)

        def seg_of(t):
            return max(s for s in SEGS if s <= t)

        def wait(ref, sem):
            if prof:
                with jax.named_scope('W'):
                    pltpu.make_async_copy(ref, ref, sem).wait()
            else:
                pltpu.make_async_copy(ref, ref, sem).wait()

        pos = [0]

        issued = set()

        def point(n0, j=0):
            for u, lag in seq:
                t = n0 - lag
                if 0 <= t < T_END and (t, u) not in issued:
                    s = seg_of(t)
                    copy(s, t - s, j, u).start(priority=pat[u])
                    if s == T_O:
                        issued.add((t, u))

        def loop(trips, body, carry=None, per=8):
            lo, hi = pos[0], pos[0] + trips * per
            edges = {s + l for s in SEGS for _, l in seq for c in (s + l,) if lo < c < hi}
            cuts = {0, trips} | {(c - lo) // per for c in edges} | {-((lo - c) // per) for c in edges}
            cuts |= {k for k in range(trips) if lo + (k + 1) * per > T_O}
            cuts = sorted(cuts)
            for a, b in zip(cuts[:-1], cuts[1:]):
                def it(k, carry, a=a):
                    for v in range(per):
                        point(lo + a * per + v, k * per)
                    return body(a + k, carry)

                carry = it(0, carry) if b - a == 1 else lax.fori_loop(0, b - a, it, carry)
            pos[0] = hi
            return carry

        def advance(n):
            if n - pos[0] >= 8:
                loop((n - pos[0]) // 2, lambda k, c: None, per=2)
            while pos[0] < n:
                point(pos[0])
                pos[0] += 1

        x_copy = pltpu.make_async_copy(x_hbm, x_buf, sem_small.at[0])
        b1_copy = pltpu.make_async_copy(b1_hbm, b1_buf, sem_small.at[1])
        b2_copy = pltpu.make_async_copy(b2_hbm, b2_buf, sem_small.at[1])
        for i in range(LAG + 2):
            advance(i + 1)
            if i == xat:
                x_copy.start()
                b1_copy.start()
                b2_copy.start()
        advance(LEAD)

        x_copy.wait()
        x = x_buf[...].astype(F32)
        xc = x - jnp.mean(x, axis=-1, keepdims=True)
        var = jnp.mean(xc * xc, axis=-1, keepdims=True)
        xn = (xc * lax.rsqrt(var + 1e-5)).astype(BF16)

        def pack(lo, hi):
            lo = lax.bitcast_convert_type(lo.astype(BF16).astype(F32), U32)
            hi = lax.bitcast_convert_type(hi.astype(BF16).astype(F32), U32)
            return (lo >> 16) | hi

        coef_ref[...] = jnp.broadcast_to(pack(xn[0:1], xn[1:2]), (H, M))

        advance(T_Q + LEAD)
        b1_copy.wait()
        b2_copy.wait()
        wait(w1_buf, sem_small.at[2])
        h = jnp.dot(xn, w1_buf[...], preferred_element_type=F32) + b1_buf[...].astype(F32).reshape(1, F)
        h = jax.nn.gelu(h, approximate=True).astype(BF16)

        lane = lax.broadcasted_iota(jnp.int32, (16, 128), 1)
        diag = (lane % 16) == lax.broadcasted_iota(jnp.int32, (16, 128), 0)

        def head_contract(seg, buf, per):
            def body(g, out):
                wait(buf.at[:, :, pl.ds(g * 16, 16)], gsem(seg, g))
                if dma_only:
                    return out
                res = []
                for hg in range(2):
                    a = []
                    for r in range(8):
                        cw = coef_ref[hg * 16:(hg + 1) * 16, (r // 2) * 128:(r // 2 + 1) * 128]
                        for t in range(2):
                            rep = jnp.take_along_axis(cw, lane // 16 + ((r % 2) * 64 + g * 16 + t * 8), axis=1)
                            a.append(jnp.where(diag, rep, jnp.uint32(0)))
                    sel = pltpu.bitcast(jnp.concatenate(a, axis=1), BF16)
                    w = buf[:, :, pl.ds(g * 16, 16), hg * 16:(hg + 1) * 16, :].reshape(2048, D)
                    res.append(out[hg] + jnp.dot(sel, w, preferred_element_type=F32))
                return tuple(res)

            advance(seg + LEAD)
            return loop(4, body, (jnp.zeros((32, D), F32), jnp.zeros((32, D), F32)), per=per)

        q = [v.astype(BF16) for v in head_contract(T_Q, wq_buf, 16 if pair else 8)]

        lane32 = lax.broadcasted_iota(jnp.int32, (32, 128), 1)
        pick = (lane32 % 8) * 16 + lax.broadcasted_iota(jnp.int32, (32, 128), 0) // 2
        q_ref[...] = jnp.zeros(q_ref.shape, F32)

        def qa_body(g, _):
            wait(wuk_buf.at[:, :, pl.ds(g * 16, 16)], gsem(T_UK, g))
            if dma_only:
                return
            for hg in range(2):
                w = wuk_buf[:, :, pl.ds(g * 16, 16), hg * 16:(hg + 1) * 16, :].reshape(2048, D)
                res = lax.dot_general(q[hg], w, NT, preferred_element_type=F32)
                for j in range(4):
                    val = q_ref[j, hg * 32:(hg + 1) * 32, :]
                    for t in range(4):
                        rep = jnp.take_along_axis(res[:, (j * 4 + t) * 128:(j * 4 + t + 1) * 128], pick, axis=1)
                        val = jnp.where(lane32 // 8 == (t // 2) * 8 + g * 2 + t % 2, rep, val)
                    q_ref[j, hg * 32:(hg + 1) * 32, :] = val

        loop(4, qa_body, per=4 if pair else 8)
        for j in range(4):
            for b in range(B):
                qa_ref[b * H:(b + 1) * H, j * 128:(j + 1) * 128] = (
                    q_ref[j, pl.ds(b, H, stride=2), :] * (D ** -0.5 * LOG2E)).astype(BF16)

        m_ref[...] = jnp.full((B * H, 128), -jnp.inf, F32)
        l_ref[...] = jnp.zeros((B * H, 128), F32)
        acc_ref[...] = jnp.zeros((B * H, DC), F32)

        def attend(g, _):
            wait(c_buf.at[pl.ds(g * 8, 8)], gsem(T_C, g))
            if dma_only:
                return
            hrows = pl.ds(al((g >> 4) * H, H), H)
            c = c_buf[pl.ds(g * 8, 8)].reshape(1024, DC)
            sc = lax.dot_general(qa_ref[hrows, :], c, NT, preferred_element_type=F32)
            m_prev = m_ref[hrows, :]
            m_new = jnp.maximum(m_prev, jnp.max(sc, axis=1, keepdims=True))
            p = jnp.exp2(sc - m_new[:, :1])
            alpha = jnp.exp2(m_prev - m_new)
            l_ref[hrows, :] = alpha * l_ref[hrows, :] + jnp.sum(p, axis=1, keepdims=True)
            m_ref[hrows, :] = m_new
            pv = jnp.dot(p.astype(BF16), c, preferred_element_type=F32)
            acc_ref[hrows, :] = acc_ref[hrows, :] * alpha[:, :1] + pv

        assert pos[0] >= T_C + LEAD
        loop(32, attend)
        pc = acc_ref[...] / l_ref[...][:, :1]
        coef_ref[...] = pack(pc[:H], pc[H:])

        advance(T_UV + LEAD)
        wait(w2_buf, sem_small.at[2])
        gg = b2_buf[...].astype(F32).reshape(1, M) + jnp.dot(h, w2_buf[...].reshape(F, M), preferred_element_type=F32)
        gate = gg * jax.nn.sigmoid(gg)

        ctx = head_contract(T_UV, wuv_buf, 8)
        ctx_ref[0:32, :] = ctx[0]
        ctx_ref[32:64, :] = ctx[1]

        advance(min(pos[0] + 3, T_END))
        lane8 = lax.broadcasted_iota(jnp.int32, (8, 128), 1)
        reg = lax.broadcasted_iota(jnp.int32, (8, 128), 0)
        slot = (lane8 // 16) == (reg % 4) * 2 + reg // 4
        for hh in range(4):
            for b in range(B):
                rows = ctx_ref[pl.ds(2 * hh + b, 8, stride=8), :]
                for dd in range(8):
                    rep = jnp.take_along_axis(rows, lane8 % 16 + dd * 16, axis=1)
                    lhs_ref[hh * 8 + dd, pl.ds(b, 1), :] = jnp.sum(jnp.where(slot, rep, 0.0), axis=0, keepdims=True)
        for i in range(NV):
            for b in range(B):
                row = lhs_ref[32 - NV + i, pl.ds(b, 1), :].astype(BF16).astype(F32)
                col_ref[i, b] = jnp.broadcast_to(row, (128, 128)).T
        advance(T_END)

        s = jnp.zeros((B, M), F32)
        for k, n in enumerate(tail_groups):
            i = o_off[k]
            advance(T_O + i + n + LAG)
            wait(wo_buf.at[i:i + n], sem_o.at[k])
            advance(min(T_O + i + n + A0 + LAG, T_END + LAG, pos[0] + n + 1))
            a = jnp.concatenate([lhs_ref[i + t] for t in range(n)], axis=1).astype(BF16)
            s = s + jnp.dot(a, wo_buf[i:i + n].reshape(128 * n, M), preferred_element_type=F32)
        nxt = [(pos[0] - LAG - T_O) * 4]

        def top_up(j):
            while nxt[0] < min(j, 128):
                i, u = divmod(nxt[0], 4)
                if (T_O + i, u) not in issued:
                    issued.add((T_O + i, u))
                    copy(T_O, i, 0, u).start(priority=0)
                nxt[0] += 1

        assert pos[0] >= T_END
        if not DV:
            top_up(128)
        if NV:
            base = x + s * gate
            base8, gate8 = (jnp.concatenate([v, jnp.zeros((6, M), F32)], axis=0) for v in (base, gate))
            acc = [jnp.zeros((8, M), F32)] * B
            for i in range(NV):
                for u in range(4):
                    j = (32 - NV + i) * 4 + u
                    top_up(j + 1)
                    wait(wo_buf.at[32 - NV + i, u], sem_v.at[i * 4 + u])
                    top_up(min(j + DV, nxt[0] + 2))
                    w = wo_buf[32 - NV + i, u].reshape(32, M).astype(F32)
                    for b in range(B):
                        su, si = order[j]
                        col = jnp.concatenate([col_ref[si - 32 + NV, b, su * 32:(su + 1) * 32, :]] * 4, axis=1)
                        pr = w * col
                        acc[b] = acc[b] + ((pr[0:8] + pr[8:16]) + (pr[16:24] + pr[24:32]))
            odd = lax.broadcasted_iota(jnp.int32, (8, M), 0) % 2 == 1
            t = jnp.where(odd, acc[1], acc[0]) + pltpu.roll(jnp.where(odd, acc[0], acc[1]), 1, 0)
            t = t + pltpu.roll(t, 4, 0)
            t = t + pltpu.roll(t, 2, 0)
            if epi:
                o_ref[...] = (base8 + t * gate8)[0:2].astype(BF16)
            else:
                o_ref[...] = (base + t[0:2] * gate).astype(BF16)
        else:
            o_ref[...] = (x + s * gate).astype(BF16)

    def outer(*refs):
        pl.run_scoped(lambda *sems: _kernel(*refs, *sems),
                      pltpu.SemaphoreType.DMA((16,)), pltpu.SemaphoreType.DMA((len(tail_groups),)),
                      pltpu.SemaphoreType.DMA((max(4 * NV, 1),)), pltpu.SemaphoreType.DMA((3,)))

    def fn(A_x, A_c_kv, A_w_q, A_w_uk, A_w_uv, A_w_o, B_x, B_w1, B_b1, B_w2, B_b2):
        wshape = (2, 4, 64, H, D)
        out = pl.pallas_call(
            outer,
            out_shape=jax.ShapeDtypeStruct((B, M), BF16),
            in_specs=[pl.BlockSpec(memory_space=pltpu.HBM)] * 10,
            out_specs=pl.BlockSpec(memory_space=pltpu.VMEM),
            scratch_shapes=[
                pltpu.VMEM((B, M), BF16), pltpu.VMEM((F,), BF16), pltpu.VMEM((M,), BF16),
                pltpu.VMEM((256, 4, 2, 16, DC), BF16),
                pltpu.VMEM(wshape, BF16), pltpu.VMEM(wshape, BF16), pltpu.VMEM(wshape, BF16),
                pltpu.VMEM((32, 4, 2, 16, M), BF16), pltpu.VMEM((M, F), BF16), pltpu.VMEM((2, 4, 224, M), BF16),
                pltpu.VMEM((H, DC), U32), pltpu.VMEM((4, B * H + 8, 128), F32),
                pltpu.VMEM((B * H, DC), BF16), pltpu.VMEM((B * H, DC), F32),
                pltpu.VMEM((B * H, 128), F32), pltpu.VMEM((B * H, 128), F32),
                pltpu.VMEM((B * H + 8, D), F32), pltpu.VMEM((32, B, 128), F32),
                pltpu.VMEM((max(NV, 1), B, 128, 128), F32),
            ],
            compiler_params=pltpu.CompilerParams(vmem_limit_bytes=100 * 1024 * 1024),
        )(A_x.reshape(B, M), A_c_kv.reshape(8, 2, 2048, DC), A_w_q.reshape(wshape), A_w_uk.reshape(wshape),
          A_w_uv.reshape(wshape), A_w_o.reshape(2, 4, 512, M), B_w1, B_b1, B_w2.reshape(2, 4, 224, M), B_b2)
        return out.reshape(B, 1, M)

    return fn


@jax.jit
def pallas_recurrent_scan__compressed_kv_cla__dense_activation_gelu__decode_kernel(
    A_x, A_c_kv, A_w_q, A_w_uk, A_w_uv, A_w_o, B_x, B_w1, B_b1, B_w2, B_b2
):
    return make_kernel(LEAD=30)(A_x, A_c_kv, A_w_q, A_w_uk, A_w_uv, A_w_o, B_x, B_w1, B_b1, B_w2, B_b2)
```

```python
import jax
import jax.numpy as jnp
from jax import lax
import jax.experimental.pallas as pl
import jax.experimental.pallas.tpu as pltpu

F32 = jnp.float32
BF16 = jnp.bfloat16
U32 = jnp.uint32

B, H, SK, D, M, DC, F = 2, 32, 16384, 128, 512, 512, 1792
LOG2E = 1.4426950408889634
NT = (((1,), (1,)), ((), ()))

T_W1, T_Q, T_UK, T_C, T_W2, T_UV, T_O, T_END = 0, 16, 48, 80, 336, 350, 382, 414
SEGMENTS = (T_W1, T_Q, T_UK, T_C, T_W2, T_UV, T_O)
POINT = ((0, 0), (3, 13), (2, 0), (1, 12))
LAG = max(lag for _, lag in POINT)
LEAD = 32
GROUP = 8
O_MXU = (8, 8, 4, 2, 2)
O_VPU = 32 - sum(O_MXU)
O_AHEAD = 24


def _kernel(x_hbm, ckv_hbm, wq_hbm, wuk_hbm, wuv_hbm, wo_hbm, w1_hbm, b1_hbm, w2_hbm, b2_hbm,
            o_ref,
            x_buf, b1_buf, b2_buf, c_buf, wq_buf, wuk_buf, wuv_buf, wo_buf, w1_buf, w2_buf,
            rows_ref, qa_ref, acc_ref, m_ref, l_ref, lhs_ref, col_ref,
            sem_small, sem_w, sem_c, sem_o):
    heads = {T_Q: (wq_hbm, wq_buf, 0), T_UK: (wuk_hbm, wuk_buf, 4), T_UV: (wuv_hbm, wuv_buf, 8)}
    o_first = [sum(O_MXU[:k]) for k in range(len(O_MXU) + 1)]

    def ckv_copy(g, t, u):
        region = (g // 16) * 4 + (t % 2) * 2 + u // 2
        row = (u % 2) * 1024 + ((g % 16) * 4 + t // 2) * 16
        if not isinstance(row, int):
            row = pl.multiple_of(row, 16)
        return pltpu.make_async_copy(ckv_hbm.at[region, :, pl.ds(row, 16)], c_buf.at[g, t * 4 + u], sem_c.at[g])

    def copy(tick, u):
        seg = max(s for s in SEGMENTS if s <= tick)
        i = tick - seg
        if seg == T_C:
            return ckv_copy(i // GROUP, i % GROUP, u)
        if seg in heads:
            hbm, buf, s0 = heads[seg]
            rows = pl.ds(2 * i, 2)
            return pltpu.make_async_copy(hbm.at[:, u, rows], buf.at[:, u, rows], sem_w.at[s0 + i // GROUP])
        if seg == T_W1:
            rows = pl.ds(((i % 2) * 4 + u) * 64 + (i // 2) * 8, 8)
            return pltpu.make_async_copy(w1_hbm.at[rows], w1_buf.at[rows], sem_small.at[2])
        rows = pl.ds(16 * i, 16)
        if seg == T_W2:
            return pltpu.make_async_copy(w2_hbm.at[:, u, rows], w2_buf.at[:, u, rows], sem_small.at[3])
        if i < o_first[-1]:
            s = max(k for k, first in enumerate(o_first) if first <= i)
        else:
            s = len(O_MXU) + (i - o_first[-1]) * 4 + u
        return pltpu.make_async_copy(wo_hbm.at[:, u, rows], wo_buf.at[i, u], sem_o.at[s])

    started = [False] * (4 * T_END)
    cursor = [0]

    def start(tick, u):
        if 0 <= tick < T_END and not started[4 * tick + u]:
            started[4 * tick + u] = True
            copy(tick, u).start(priority=1 - u % 2)

    def advance(point):
        for n in range(cursor[0], min(point, T_END)):
            for u, lag in POINT:
                start(n - lag, u)
        cursor[0] = max(cursor[0], point)

    pending = [0]

    def release(upto, most):
        while pending[0] < min(upto, 4 * T_END) and (most > 0 or started[pending[0]]):
            most -= not started[pending[0]]
            start(pending[0] // 4, pending[0] % 4)
            pending[0] += 1

    def wait(slab, sem, first, last):
        assert all(started[first:last])
        pltpu.make_async_copy(slab, slab, sem).wait()

    x_copy = pltpu.make_async_copy(x_hbm, x_buf, sem_small.at[0])
    b1_copy = pltpu.make_async_copy(b1_hbm, b1_buf, sem_small.at[1])
    b2_copy = pltpu.make_async_copy(b2_hbm, b2_buf, sem_small.at[1])
    advance(2)
    x_copy.start()
    b1_copy.start()
    b2_copy.start()
    advance(LEAD)

    x_copy.wait()
    x = x_buf[...].astype(F32)
    xc = x - jnp.mean(x, axis=-1, keepdims=True)
    var = jnp.mean(xc * xc, axis=-1, keepdims=True)
    xn = (xc * lax.rsqrt(var + 1e-5)).astype(BF16)

    advance(T_Q + LEAD)
    b1_copy.wait()
    b2_copy.wait()
    wait(w1_buf, sem_small.at[2], 4 * T_W1, 4 * T_Q)
    h = jnp.dot(xn, w1_buf[...], preferred_element_type=F32) + b1_buf[...].astype(F32).reshape(1, F)
    h = jax.nn.gelu(h, approximate=True).astype(BF16)

    def head_tiles(seg):
        _, buf, s0 = heads[seg]
        for g in range(4):
            first = seg + g * GROUP
            advance(first + GROUP + LEAD)
            wait(buf.at[:, :, pl.ds(16 * g, 16)], sem_w.at[s0 + g], 4 * first, 4 * (first + GROUP))
            for hg in range(2):
                yield g, hg, buf[:, :, pl.ds(16 * g, 16), pl.ds(16 * hg, 16), :].reshape(16 * 128, D)

    lane = lax.broadcasted_iota(jnp.int32, (16, 128), 1)
    diag = lane % 16 == lax.broadcasted_iota(jnp.int32, (16, 128), 0)

    def head_contract(seg, coef0, coef1):
        lo, hi = (lax.bitcast_convert_type(c.astype(BF16).astype(F32), U32) for c in (coef0, coef1))
        words = (lo >> 16) | hi
        out = [jnp.zeros((16 * B, D), F32)] * 2
        for g, hg, w in head_tiles(seg):
            lhs = []
            for t in range(16):
                c0 = 64 * (t // 2) + 16 * g + 8 * (t % 2)
                src = words[16 * hg:16 * (hg + 1), c0 // 128 * 128:(c0 // 128 + 1) * 128]
                rep = jnp.take_along_axis(src, lane // 16 + c0 % 128, axis=1)
                lhs.append(jnp.where(diag, rep, jnp.zeros_like(rep)))
            lhs = pltpu.bitcast(jnp.concatenate(lhs, axis=1), BF16)
            out[hg] = out[hg] + jnp.dot(lhs, w, preferred_element_type=F32)
        return out

    q = head_contract(T_Q, jnp.broadcast_to(xn[0:1].astype(F32), (H, M)), jnp.broadcast_to(xn[1:2].astype(F32), (H, M)))
    q = [v.astype(BF16) for v in q]

    lane32 = lax.broadcasted_iota(jnp.int32, (16 * B, 128), 1)
    own = (lane32 % 8) * 16 + lax.broadcasted_iota(jnp.int32, (16 * B, 128), 0) // 2
    rows_ref[...] = jnp.zeros(rows_ref.shape, F32)
    for g, hg, w in head_tiles(T_UK):
        r = lax.dot_general(q[hg], w, NT, preferred_element_type=F32)
        for j in range(DC // 128):
            val = rows_ref[j, pl.ds(32 * hg, 32), :]
            for t in range(4 * j, 4 * j + 4):
                c0 = 64 * (t // 2) + 16 * g + 8 * (t % 2)
                rep = jnp.take_along_axis(r[:, 128 * t:128 * (t + 1)], own, axis=1)
                val = jnp.where(lane32 // 8 == c0 % 128 // 8, rep, val)
            rows_ref[j, pl.ds(32 * hg, 32), :] = val
    for j in range(DC // 128):
        for b in range(B):
            qa = rows_ref[j, pl.ds(b, H, stride=B), :] * (D ** -0.5 * LOG2E)
            qa_ref[b, :, 128 * j:128 * (j + 1)] = qa.astype(BF16)

    m_ref[...] = jnp.full(m_ref.shape, -jnp.inf, F32)
    l_ref[...] = jnp.zeros(l_ref.shape, F32)
    acc_ref[...] = jnp.zeros(acc_ref.shape, F32)

    def attend(g):
        b = g // 16
        c = c_buf[g].reshape(GROUP * 128, DC)
        sc = lax.dot_general(qa_ref[b], c, NT, preferred_element_type=F32)
        m_prev = m_ref[b]
        m_new = jnp.maximum(m_prev, jnp.max(sc, axis=1, keepdims=True))
        p = jnp.exp2(sc - m_new[:, :1])
        alpha = jnp.exp2(m_prev - m_new)
        l_ref[b] = alpha * l_ref[b] + jnp.sum(p, axis=1, keepdims=True)
        m_ref[b] = m_new
        acc_ref[b] = acc_ref[b] * alpha[:, :1] + jnp.dot(p.astype(BF16), c, preferred_element_type=F32)

    ahead = LEAD // GROUP
    rolled = 32 - ahead
    assert cursor[0] == T_C + ahead * GROUP

    def step(g, _):
        for v in range(GROUP):
            for u, lag in POINT:
                ckv_copy(g + ahead + (v - lag) // GROUP, (v - lag) % GROUP, u).start(priority=1 - u % 2)
        pltpu.make_async_copy(c_buf.at[g], c_buf.at[g], sem_c.at[g]).wait()
        attend(g)

    lax.fori_loop(0, rolled, step, None)
    for n in range(cursor[0], T_W2):
        for u, lag in POINT:
            started[4 * (n - lag) + u] = True
    cursor[0] = T_W2
    for g in range(rolled, 32):
        first = T_C + g * GROUP
        advance(first + GROUP + LEAD)
        wait(c_buf.at[g], sem_c.at[g], 4 * first, 4 * (first + GROUP))
        attend(g)

    advance(T_UV + LEAD)
    wait(w2_buf, sem_small.at[3], 4 * T_W2, 4 * T_UV)
    gate = jnp.dot(h, w2_buf[...].reshape(F, M), preferred_element_type=F32) + b2_buf[...].astype(F32).reshape(1, M)
    gate = gate * jax.nn.sigmoid(gate)

    ctx = head_contract(T_UV, *(acc_ref[b] / l_ref[b][:, :1] for b in range(B)))
    rows_ref[0, 0:32, :] = ctx[0]
    rows_ref[0, 32:64, :] = ctx[1]

    lane8 = lax.broadcasted_iota(jnp.int32, (8, 128), 1)
    region = lax.broadcasted_iota(jnp.int32, (8, 128), 0)
    slot = lane8 // 16 == (region % 4) * 2 + region // 4
    for hh in range(4):
        for b in range(B):
            src = rows_ref[0, pl.ds(B * hh + b, 8, stride=4 * B), :]
            for dd in range(8):
                rep = jnp.take_along_axis(src, lane8 % 16 + 16 * dd, axis=1)
                lhs_ref[8 * hh + dd, pl.ds(b, 1), :] = jnp.sum(jnp.where(slot, rep, 0.0), axis=0, keepdims=True)
    for i in range(O_VPU):
        for b in range(B):
            row = lhs_ref[o_first[-1] + i, pl.ds(b, 1), :].astype(BF16).astype(F32)
            col_ref[i, b] = jnp.broadcast_to(row, (128, 128)).T

    assert cursor[0] >= T_END
    s = jnp.zeros((B, M), F32)
    for k, n in enumerate(O_MXU):
        i = o_first[k]
        last = 4 * (T_O + i + n)
        release(last, 4 * n)
        wait(wo_buf.at[pl.ds(i, n)], sem_o.at[k], last - 4 * n, last)
        release(last + O_AHEAD, 2 * n + 2)
        lhs = jnp.concatenate([lhs_ref[i + t] for t in range(n)], axis=1).astype(BF16)
        s = s + jnp.dot(lhs, wo_buf[pl.ds(i, n)].reshape(128 * n, M), preferred_element_type=F32)

    fill = jnp.zeros((8 - B, M), F32)
    base = jnp.concatenate([x + s * gate, fill], axis=0)
    gate = jnp.concatenate([gate, fill], axis=0)
    part = [jnp.zeros((8, M), F32)] * B
    for j in range(4 * O_VPU):
        i, u = divmod(j, 4)
        at = 4 * (T_O + o_first[-1]) + j
        release(at + 1, 1)
        piece = wo_buf.at[o_first[-1] + i, u]
        wait(piece, sem_o.at[len(O_MXU) + j], at, at + 1)
        release(at + O_AHEAD, 1)
        w = piece[...].reshape(32, M).astype(F32)
        for b in range(B):
            pr = w * jnp.concatenate([col_ref[i, b, pl.ds(32 * u, 32), :]] * (M // 128), axis=1)
            part[b] = part[b] + ((pr[0:8] + pr[8:16]) + (pr[16:24] + pr[24:32]))
    assert all(started)
    odd = lax.broadcasted_iota(jnp.int32, (8, M), 0) % 2 == 1
    total = jnp.where(odd, part[1], part[0]) + pltpu.roll(jnp.where(odd, part[0], part[1]), 1, 0)
    total = total + pltpu.roll(total, 4, 0)
    total = total + pltpu.roll(total, 2, 0)
    o_ref[...] = (base + total * gate)[0:B].astype(BF16)


def _kernel_with_semaphores(*refs):
    pl.run_scoped(lambda *sems: _kernel(*refs, *sems),
                  pltpu.SemaphoreType.DMA((4,)), pltpu.SemaphoreType.DMA((12,)), pltpu.SemaphoreType.DMA((32,)),
                  pltpu.SemaphoreType.DMA((len(O_MXU) + 4 * O_VPU,)))


@jax.jit
def pallas_recurrent_scan__compressed_kv_cla__dense_activation_gelu__decode_kernel(
    A_x: jax.Array,
    A_c_kv: jax.Array,
    A_w_q: jax.Array,
    A_w_uk: jax.Array,
    A_w_uv: jax.Array,
    A_w_o: jax.Array,
    B_x: jax.Array,
    B_w1: jax.Array,
    B_b1: jax.Array,
    B_w2: jax.Array,
    B_b2: jax.Array,
):
    del B_x
    head_shape = (2, 4, 64, H, D)
    w2_shape = (2, 4, F // 8, M)
    out = pl.pallas_call(
        _kernel_with_semaphores,
        out_shape=jax.ShapeDtypeStruct((B, M), BF16),
        in_specs=[pl.BlockSpec(memory_space=pltpu.HBM)] * 10,
        out_specs=pl.BlockSpec(memory_space=pltpu.VMEM),
        scratch_shapes=[
            pltpu.VMEM((B, M), BF16), pltpu.VMEM((F,), BF16), pltpu.VMEM((M,), BF16),
            pltpu.VMEM((32, 4 * GROUP, 2, 16, DC), BF16),
            pltpu.VMEM(head_shape, BF16), pltpu.VMEM(head_shape, BF16), pltpu.VMEM(head_shape, BF16),
            pltpu.VMEM((32, 4, 2, 16, M), BF16), pltpu.VMEM((M, F), BF16), pltpu.VMEM(w2_shape, BF16),
            pltpu.VMEM((DC // 128, B * H + 8, 128), F32), pltpu.VMEM((B, H, DC), BF16),
            pltpu.VMEM((B, H, DC), F32), pltpu.VMEM((B, H, 128), F32), pltpu.VMEM((B, H, 128), F32),
            pltpu.VMEM((32, B, 128), F32), pltpu.VMEM((O_VPU, B, 128, 128), F32),
        ],
        compiler_params=pltpu.CompilerParams(vmem_limit_bytes=100 * 1024 * 1024),
    )(A_x.reshape(B, M), A_c_kv.reshape(8, 2, SK // 8, DC), A_w_q.reshape(head_shape), A_w_uk.reshape(head_shape),
      A_w_uv.reshape(head_shape), A_w_o.reshape(2, 4, H * D // 8, M), B_w1, B_b1, B_w2.reshape(w2_shape), B_b2)
    return out.reshape(B, 1, M)
```

```python
import jax
import jax.numpy as jnp
from jax import lax
import jax.experimental.pallas as pl
import jax.experimental.pallas.tpu as pltpu

F32 = jnp.float32
BF16 = jnp.bfloat16
U32 = jnp.uint32

B, H, SK, D, M, DC, F = 2, 32, 16384, 128, 512, 512, 1792
LOG2E = 1.4426950408889634
NT = (((1,), (1,)), ((), ()))

T_W1, T_Q, T_UK, T_C, T_W2, T_UV, T_O, T_END = 0, 16, 48, 80, 336, 350, 382, 414
SEGMENTS = (T_W1, T_Q, T_UK, T_C, T_W2, T_UV, T_O)
POINT = ((0, 0), (3, 13), (2, 0), (1, 12))
LEAD = 32
GROUP = 8
O_MXU = (8, 8)
O_VPU = 32 - sum(O_MXU)
O_AHEAD = 28
O_EARLY = 6


def _kernel(x_hbm, ckv_hbm, wq_hbm, wuk_hbm, wuv_hbm, wo_hbm, w1_hbm, b1_hbm, w2_hbm, b2_hbm,
            o_ref,
            x_buf, b1_buf, b2_buf, c_buf, wq_buf, wuk_buf, wuv_buf, wo_buf, w1_buf, w2_buf,
            rows_ref, qa_ref, acc_ref, m_ref, l_ref, lhs_ref, col_ref,
            sem_small, sem_w, sem_c, sem_o):
    heads = {T_Q: (wq_hbm, wq_buf, 0), T_UK: (wuk_hbm, wuk_buf, 4), T_UV: (wuv_hbm, wuv_buf, 8)}
    o_first = [sum(O_MXU[:k]) for k in range(len(O_MXU) + 1)]

    def ckv_copy(g, t, u):
        region = (g // 16) * 4 + (t % 2) * 2 + u // 2
        row = (u % 2) * 1024 + ((g % 16) * 4 + t // 2) * 16
        if not isinstance(row, int):
            row = pl.multiple_of(row, 16)
        return pltpu.make_async_copy(ckv_hbm.at[region, :, pl.ds(row, 16)], c_buf.at[g, t * 4 + u], sem_c.at[g])

    def copy(tick, u):
        seg = max(s for s in SEGMENTS if s <= tick)
        i = tick - seg
        if seg == T_C:
            return ckv_copy(i // GROUP, i % GROUP, u)
        if seg in heads:
            hbm, buf, s0 = heads[seg]
            rows = pl.ds(2 * i, 2)
            return pltpu.make_async_copy(hbm.at[:, u, rows], buf.at[:, u, rows], sem_w.at[s0 + i // GROUP])
        if seg == T_W1:
            rows = pl.ds(128 * u + 8 * i, 8)
            return pltpu.make_async_copy(w1_hbm.at[rows], w1_buf.at[rows], sem_small.at[2])
        rows = pl.ds(16 * i, 16)
        if seg == T_W2:
            return pltpu.make_async_copy(w2_hbm.at[:, u, rows], w2_buf.at[:, u, rows], sem_small.at[3])
        if i < o_first[-1]:
            s = max(k for k, first in enumerate(o_first) if first <= i)
        else:
            s = len(O_MXU) + (i - o_first[-1]) * 4 + u
        return pltpu.make_async_copy(wo_hbm.at[:, u, rows], wo_buf.at[i, u], sem_o.at[s])

    started = [False] * (4 * T_END)
    cursor = [0]

    def start(tick, u):
        if 0 <= tick < T_END and not started[4 * tick + u]:
            started[4 * tick + u] = True
            copy(tick, u).start(priority=1 - u % 2)

    def advance(point):
        for n in range(cursor[0], min(point, T_END)):
            for u, lag in POINT:
                start(n - lag, u)
        cursor[0] = max(cursor[0], point)

    pending = [0]

    def release(upto, most):
        while pending[0] < min(upto, 4 * T_END) and (most > 0 or started[pending[0]]):
            most -= not started[pending[0]]
            start(pending[0] // 4, pending[0] % 4)
            pending[0] += 1

    def wait(slab, sem, first, last):
        assert all(started[first:last])
        pltpu.make_async_copy(slab, slab, sem).wait()

    x_copy = pltpu.make_async_copy(x_hbm, x_buf, sem_small.at[0])
    b1_copy = pltpu.make_async_copy(b1_hbm, b1_buf, sem_small.at[1])
    b2_copy = pltpu.make_async_copy(b2_hbm, b2_buf, sem_small.at[1])
    advance(2)
    x_copy.start()
    b1_copy.start()
    b2_copy.start()
    advance(LEAD)

    x_copy.wait()
    x = x_buf[...].astype(F32)
    xc = x - jnp.mean(x, axis=-1, keepdims=True)
    var = jnp.mean(xc * xc, axis=-1, keepdims=True)
    xn = (xc * lax.rsqrt(var + 1e-5)).astype(BF16)

    advance(T_Q + LEAD)
    b1_copy.wait()
    b2_copy.wait()
    wait(w1_buf, sem_small.at[2], 4 * T_W1, 4 * T_Q)
    h = jnp.dot(xn, w1_buf[...], preferred_element_type=F32) + b1_buf[...].astype(F32).reshape(1, F)
    h = jax.nn.gelu(h, approximate=True).astype(BF16)

    def head_tiles(seg):
        _, buf, s0 = heads[seg]
        for g in range(4):
            first = seg + g * GROUP
            advance(first + GROUP + LEAD)
            wait(buf.at[:, :, pl.ds(16 * g, 16)], sem_w.at[s0 + g], 4 * first, 4 * (first + GROUP))
            for hg in range(2):
                yield g, hg, buf[:, :, pl.ds(16 * g, 16), pl.ds(16 * hg, 16), :].reshape(16 * 128, D)

    lane = lax.broadcasted_iota(jnp.int32, (16, 128), 1)
    diag = lane % 16 == lax.broadcasted_iota(jnp.int32, (16, 128), 0)

    def head_contract(seg, coef0, coef1):
        lo, hi = (lax.bitcast_convert_type(c.astype(BF16).astype(F32), U32) for c in (coef0, coef1))
        words = (lo >> 16) | hi
        out = [jnp.zeros((16 * B, D), F32)] * 2
        for g, hg, w in head_tiles(seg):
            lhs = []
            for t in range(16):
                c0 = 64 * (t // 2) + 16 * g + 8 * (t % 2)
                src = words[16 * hg:16 * (hg + 1), c0 // 128 * 128:(c0 // 128 + 1) * 128]
                rep = jnp.take_along_axis(src, lane // 16 + c0 % 128, axis=1)
                lhs.append(jnp.where(diag, rep, jnp.zeros_like(rep)))
            lhs = pltpu.bitcast(jnp.concatenate(lhs, axis=1), BF16)
            out[hg] = out[hg] + jnp.dot(lhs, w, preferred_element_type=F32)
        return out

    q = head_contract(T_Q, jnp.broadcast_to(xn[0:1].astype(F32), (H, M)), jnp.broadcast_to(xn[1:2].astype(F32), (H, M)))
    q = [v.astype(BF16) for v in q]

    lane32 = lax.broadcasted_iota(jnp.int32, (16 * B, 128), 1)
    own = (lane32 % 8) * 16 + lax.broadcasted_iota(jnp.int32, (16 * B, 128), 0) // 2
    rows_ref[...] = jnp.zeros(rows_ref.shape, F32)
    for g, hg, w in head_tiles(T_UK):
        r = lax.dot_general(q[hg], w, NT, preferred_element_type=F32)
        for j in range(DC // 128):
            val = rows_ref[j, pl.ds(32 * hg, 32), :]
            for t in range(4 * j, 4 * j + 4):
                c0 = 64 * (t // 2) + 16 * g + 8 * (t % 2)
                rep = jnp.take_along_axis(r[:, 128 * t:128 * (t + 1)], own, axis=1)
                val = jnp.where(lane32 // 8 == c0 % 128 // 8, rep, val)
            rows_ref[j, pl.ds(32 * hg, 32), :] = val
    for j in range(DC // 128):
        for b in range(B):
            qa = rows_ref[j, pl.ds(b, H, stride=B), :] * (D ** -0.5 * LOG2E)
            qa_ref[b, :, 128 * j:128 * (j + 1)] = qa.astype(BF16)

    m_ref[...] = jnp.full(m_ref.shape, -jnp.inf, F32)
    l_ref[...] = jnp.zeros(l_ref.shape, F32)
    acc_ref[...] = jnp.zeros(acc_ref.shape, F32)

    def attend(g):
        b = g // 16
        c = c_buf[g].reshape(GROUP * 128, DC)
        sc = lax.dot_general(qa_ref[b], c, NT, preferred_element_type=F32)
        m_prev = m_ref[b]
        m_new = jnp.maximum(m_prev, jnp.max(sc, axis=1, keepdims=True))
        p = jnp.exp2(sc - m_new[:, :1])
        alpha = jnp.exp2(m_prev - m_new)
        l_ref[b] = alpha * l_ref[b] + jnp.sum(p, axis=1, keepdims=True)
        m_ref[b] = m_new
        acc_ref[b] = acc_ref[b] * alpha[:, :1] + jnp.dot(p.astype(BF16), c, preferred_element_type=F32)

    ahead = LEAD // GROUP
    rolled = 32 - ahead
    assert cursor[0] == T_C + ahead * GROUP

    def step(g, _):
        for v in range(GROUP):
            for u, lag in POINT:
                ckv_copy(g + ahead + (v - lag) // GROUP, (v - lag) % GROUP, u).start(priority=1 - u % 2)
        pltpu.make_async_copy(c_buf.at[g], c_buf.at[g], sem_c.at[g]).wait()
        attend(g)

    lax.fori_loop(0, rolled, step, None)
    for n in range(cursor[0], T_W2):
        for u, lag in POINT:
            started[4 * (n - lag) + u] = True
    cursor[0] = T_W2
    for g in range(rolled, 32):
        first = T_C + g * GROUP
        advance(first + GROUP + LEAD)
        wait(c_buf.at[g], sem_c.at[g], 4 * first, 4 * (first + GROUP))
        attend(g)

    advance(T_UV + LEAD)
    wait(w2_buf, sem_small.at[3], 4 * T_W2, 4 * T_UV)
    gate = jnp.dot(h, w2_buf[...].reshape(F, M), preferred_element_type=F32) + b2_buf[...].astype(F32).reshape(1, M)
    gate = gate * jax.nn.sigmoid(gate)

    ctx = head_contract(T_UV, *(acc_ref[b] / l_ref[b][:, :1] for b in range(B)))
    rows_ref[0, 0:32, :] = ctx[0]
    rows_ref[0, 32:64, :] = ctx[1]

    lane8 = lax.broadcasted_iota(jnp.int32, (8, 128), 1)
    region = lax.broadcasted_iota(jnp.int32, (8, 128), 0)
    slot = lane8 // 16 == (region % 4) * 2 + region // 4
    for hh in range(4):
        for b in range(B):
            src = rows_ref[0, pl.ds(B * hh + b, 8, stride=4 * B), :]
            for dd in range(8):
                rep = jnp.take_along_axis(src, lane8 % 16 + 16 * dd, axis=1)
                lhs_ref[8 * hh + dd, pl.ds(b, 1), :] = jnp.sum(jnp.where(slot, rep, 0.0), axis=0, keepdims=True)
    for i in range(O_VPU):
        for b in range(B):
            row = lhs_ref[o_first[-1] + i, pl.ds(b, 1), :].astype(BF16).astype(F32)
            col_ref[i, b] = jnp.broadcast_to(row, (128, 128)).T

    assert cursor[0] >= T_END
    s = jnp.zeros((B, M), F32)
    for k, n in enumerate(O_MXU):
        i = o_first[k]
        last = 4 * (T_O + i + n)
        release(last, 4 * n)
        wait(wo_buf.at[pl.ds(i, n)], sem_o.at[k], last - 4 * n, last)
        release(last + O_AHEAD, 2 * n + 2)
        lhs = jnp.concatenate([lhs_ref[i + t] for t in range(n)], axis=1).astype(BF16)
        s = s + jnp.dot(lhs, wo_buf[pl.ds(i, n)].reshape(128 * n, M), preferred_element_type=F32)

    fill = jnp.zeros((8 - B, M), F32)
    base = jnp.concatenate([x + s * gate, fill], axis=0)
    gate = jnp.concatenate([gate, fill], axis=0)
    part = [jnp.zeros((8, M), F32)] * B
    for j in sorted(range(4 * O_VPU), key=lambda j: j - O_EARLY * (j % 2)):
        i, u = divmod(j, 4)
        at = 4 * (T_O + o_first[-1]) + j
        release(at + 1, 4 * O_VPU)
        piece = wo_buf.at[o_first[-1] + i, u]
        wait(piece, sem_o.at[len(O_MXU) + j], at, at + 1)
        release(at + O_AHEAD, 1 - u % 2)
        w = piece[...].reshape(32, M).astype(F32)
        for b in range(B):
            pr = w * jnp.concatenate([col_ref[i, b, pl.ds(32 * u, 32), :]] * (M // 128), axis=1)
            part[b] = part[b] + ((pr[0:8] + pr[8:16]) + (pr[16:24] + pr[24:32]))
    assert all(started)
    odd = lax.broadcasted_iota(jnp.int32, (8, M), 0) % 2 == 1
    total = jnp.where(odd, part[1], part[0]) + pltpu.roll(jnp.where(odd, part[0], part[1]), 1, 0)
    total = total + pltpu.roll(total, 4, 0)
    total = total + pltpu.roll(total, 2, 0)
    o_ref[...] = (base + total * gate)[0:B].astype(BF16)


def _kernel_with_semaphores(*refs):
    pl.run_scoped(lambda *sems: _kernel(*refs, *sems),
                  pltpu.SemaphoreType.DMA((4,)), pltpu.SemaphoreType.DMA((12,)), pltpu.SemaphoreType.DMA((32,)),
                  pltpu.SemaphoreType.DMA((len(O_MXU) + 4 * O_VPU,)))


@jax.jit
def pallas_recurrent_scan__compressed_kv_cla__dense_activation_gelu__decode_kernel(
    A_x: jax.Array,
    A_c_kv: jax.Array,
    A_w_q: jax.Array,
    A_w_uk: jax.Array,
    A_w_uv: jax.Array,
    A_w_o: jax.Array,
    B_x: jax.Array,
    B_w1: jax.Array,
    B_b1: jax.Array,
    B_w2: jax.Array,
    B_b2: jax.Array,
):
    del B_x
    head_shape = (2, 4, 64, H, D)
    w2_shape = (2, 4, F // 8, M)
    out = pl.pallas_call(
        _kernel_with_semaphores,
        out_shape=jax.ShapeDtypeStruct((B, M), BF16),
        in_specs=[pl.BlockSpec(memory_space=pltpu.HBM)] * 10,
        out_specs=pl.BlockSpec(memory_space=pltpu.VMEM),
        scratch_shapes=[
            pltpu.VMEM((B, M), BF16), pltpu.VMEM((F,), BF16), pltpu.VMEM((M,), BF16),
            pltpu.VMEM((32, 4 * GROUP, 2, 16, DC), BF16),
            pltpu.VMEM(head_shape, BF16), pltpu.VMEM(head_shape, BF16), pltpu.VMEM(head_shape, BF16),
            pltpu.VMEM((32, 4, 2, 16, M), BF16), pltpu.VMEM((M, F), BF16), pltpu.VMEM(w2_shape, BF16),
            pltpu.VMEM((DC // 128, B * H + 8, 128), F32), pltpu.VMEM((B, H, DC), BF16),
            pltpu.VMEM((B, H, DC), F32), pltpu.VMEM((B, H, 128), F32), pltpu.VMEM((B, H, 128), F32),
            pltpu.VMEM((32, B, 128), F32), pltpu.VMEM((O_VPU, B, 128, 128), F32),
        ],
        compiler_params=pltpu.CompilerParams(vmem_limit_bytes=100 * 1024 * 1024),
    )(A_x.reshape(B, M), A_c_kv.reshape(8, 2, SK // 8, DC), A_w_q.reshape(head_shape), A_w_uk.reshape(head_shape),
      A_w_uv.reshape(head_shape), A_w_o.reshape(2, 4, H * D // 8, M), B_w1, B_b1, B_w2.reshape(w2_shape), B_b2)
    return out.reshape(B, 1, M)
```
